```python
import os as _os
_os.environ.setdefault("JAX_PLATFORMS", "cpu")
import jax
import jax.numpy as jnp

def _softmax(x, axis=-1):
    return jax.nn.softmax(x, axis=axis)
def _gelu(x):
    return jax.nn.gelu(x, approximate=True)
def _silu(x):
    return jax.nn.silu(x)
def _sigmoid(x):
    return jax.nn.sigmoid(x)
def _layernorm(x, axis=-1, eps=1e-5):
    m = jnp.mean(x, axis=axis, keepdims=True)
    v = jnp.var(x, axis=axis, keepdims=True)
    return (x - m) / jnp.sqrt(v + eps)
def _scatter_add(tgt, idx, src, axis=0):
    return tgt.at[idx].add(src)
def _segment_sum(src, seg, n):
    return jax.ops.segment_sum(src, seg, n)
class _Rng:
    def __init__(self, key):
        self._k = key
    def _next(self):
        self._k, sub = jax.random.split(self._k)
        return sub
    def normal(self, shape):
        return jax.random.normal(self._next(), shape, dtype=jnp.bfloat16)
    def randint(self, lo, hi, shape):
        return jax.random.randint(self._next(), shape, lo, hi, dtype=jnp.int32)
    def uniform(self, shape, lo=0.0, hi=1.0):
        return jax.random.uniform(self._next(), shape, jnp.bfloat16, lo, hi)
    def permutation(self, n):
        return jax.random.permutation(self._next(), n)


kernel_name = 'gated_mix__sliding_block_cached__dense_activation_silu__decode'

def setup_inputs():
    _rng = _Rng(jax.random.key(int.from_bytes(__import__("os").urandom(4), "little")))
    _w = (lambda a: (lambda t: t.astype(jnp.bfloat16) if jnp.issubdtype(t.dtype, jnp.floating) else t)(jnp.asarray(a)))
    def _A_setup():
        B, Sq, D = 2, 1, 1024
        Hq, Hkv, Sk, Dh = 32, 4, 32768, 128
        assert Hq % Hkv == 0, (Hq, Hkv)
        return {
            "x": _w((lambda *s: _rng.normal(s) * 0.05)(B, Sq, D)),
            "k_cache": _w((lambda *s: _rng.normal(s) * 3.2)(B, Hkv, Sk, Dh)),
            "v_cache": _w((lambda *s: _rng.normal(s) * 0.05)(B, Hkv, Sk, Dh)),
            "wq": _w((lambda *s: _rng.normal(s) * 3.2)(D, Hq * Dh) * (D ** -0.5)),
            "wo": _w((lambda *s: _rng.normal(s) * 0.05)(Hq * Dh, D) * ((Hq * Dh) ** -0.5)),
        }
    _A_in = _A_setup()

    def _B_setup():
        B, S, D, F = 2, 1, 1024, 3584
        return {
            "x": _w((lambda *s: _rng.normal(s) * 0.05)(B, S, D)),
            "w1": _w((lambda *s: _rng.normal(s) * 0.05)(D, F) * (D ** -0.5)),
            "w2": _w((lambda *s: _rng.normal(s) * 0.05)(F, D) * (F ** -0.5)),
        }
    _B_in = _B_setup()

    return {
        "A_x": _A_in["x"],
        "A_k_cache": _A_in["k_cache"],
        "A_v_cache": _A_in["v_cache"],
        "A_wq": _A_in["wq"],
        "A_wo": _A_in["wo"],
        "B_x": _B_in["x"],
        "B_w1": _B_in["w1"],
        "B_w2": _B_in["w2"],
        "gate_w": _w((lambda *s: _rng.normal(s) * 0.05)(1024) * 16.0),
    }

def reference(A_x, A_k_cache, A_v_cache, A_wq, A_wo, B_x, B_w1, B_w2, gate_w):
    def _A_ref(x, k_cache, v_cache, wq, wo):
        B, Sq, D = x.shape
        Hq, Dh = 32, 128
        Hkv, Sk = k_cache.shape[1], k_cache.shape[2]
        W = min(4096, max(256, Sk // 4))
        rep = Hq // Hkv
        q = (lambda x, *d: x.transpose(*d))((x @ wq).reshape(B, Sq, Hq, Dh), 0, 2, 1, 3)
        k = jnp.repeat(k_cache[:, :, Sk - W:, :], rep, axis=1)
        v = jnp.repeat(v_cache[:, :, Sk - W:, :], rep, axis=1)
        scores = jnp.einsum("bhqd,bhkd->bhqk", q, k) * (Dh ** -0.5)
        p = _softmax(scores, axis=-1)
        o = jnp.einsum("bhqk,bhkd->bhqd", p, v)
        return (lambda x, *d: x.transpose(*d))(o, 0, 2, 1, 3).reshape(B, Sq, Hq * Dh) @ wo

    def _B_ref(x, w1, w2):
        h = jnp.einsum("bsd,df->bsf", x, w1)
        h = _silu(h)
        out = jnp.einsum("bsf,fd->bsd", h, w2)
        return out

    x = A_x
    g = _sigmoid((x * gate_w).sum(-1, keepdims=True))
    a = _A_ref(x, A_k_cache, A_v_cache, A_wq, A_wo)
    b = _B_ref(x, B_w1, B_w2)
    return g * a + (1 - g) * b
```

```python
import functools

import jax
import jax.numpy as jnp
from jax import lax
import jax.experimental.pallas as pl
import jax.experimental.pallas.tpu as pltpu

HQ, DH = 32, 128
F32, BF16 = jnp.float32, jnp.bfloat16


def _dot(a, b):
    return jnp.dot(a, b, preferred_element_type=F32)


def _kernel(x_h, k_h, v_h, wq_h, wo_h, w1_h, w2_h, gw_h, o_ref,
            x_v, gw_v, k_v, v_v, wq_v, wo_v, w1_v, w2_v,
            xs, acc, qs, os_, hs, sems, ssem, *, depth, rq, r1, ro, r2, compute):
    B, D = x_h.shape
    _, HKV, SK, _ = k_h.shape
    F = w1_h.shape[1]
    W = min(4096, max(256, SK // 4))
    rep = HQ // HKV
    NKV = B * HKV

    def rows(h, v, r):
        return lambda i, s: pltpu.make_async_copy(
            h.at[pl.ds(pl.multiple_of(i * r, r), r)],
            v.at[pl.ds(pl.multiple_of(i * r, r), r)], s)

    def kv(i, s):
        n = i // 2
        return [functools.partial(pltpu.make_async_copy, h.at[n // HKV, n % HKV, pl.ds(SK - W, W)], v.at[n], s)
                for h, v in ((k_h, k_v), (v_h, v_v))]

    phases = [(rows(wq_h, wq_v, rq), D // rq), (rows(w1_h, w1_v, r1), D // r1),
              (None, 2 * NKV), (rows(w2_h, w2_v, r2), F // r2),
              (rows(wo_h, wo_v, ro), HQ * DH // ro)]
    base = [0]
    for _, n in phases:
        base.append(base[-1] + n)

    def start(g, lo, hi):
        for p, (mk, n) in enumerate(phases):
            if base[p + 1] <= lo or base[p] >= hi:
                continue

            def go(p=p, mk=mk):
                i = g - base[p]
                if mk is None:
                    ck, cv = kv(i, sems.at[g])
                    if isinstance(i, int):
                        (cv if i % 2 else ck)().start()
                    else:
                        pl.when(i % 2 == 0)(lambda: ck().start())
                        pl.when(i % 2 == 1)(lambda: cv().start())
                else:
                    mk(i, sems.at[g]).start()
            if base[p] <= lo and hi <= base[p + 1]:
                go()
            else:
                pl.when((g >= base[p]) & (g < base[p + 1]))(go)

    def run(p, body, init=None, step=1):
        mk, n = phases[p]

        def it(j, c):
            for u in range(step):
                i = j * step + u
                g = base[p] + i
                cp = kv(i, sems.at[g])[u]() if mk is None else mk(i, sems.at[g])
                cp.wait()
                start(g + depth, base[p] + depth, base[p + 1] + depth)
            return body(j, c) if compute else c
        return lax.fori_loop(0, n // step, it, init)

    cx = pltpu.make_async_copy(x_h, x_v, ssem.at[0])
    cg = pltpu.make_async_copy(gw_h, gw_v, ssem.at[1])
    start(0, 0, 1)
    cx.start()
    cg.start()
    for g in range(1, depth):
        start(g, g, g + 1)
    cx.wait()
    cg.wait()
    xs[...] = jnp.zeros_like(xs)
    os_[...] = jnp.zeros_like(os_)
    xs[0:B, :] = x_v[...].astype(F32)

    def mm(lhs, w, r, n):
        acc[:, :n] = jnp.zeros((8, n), F32)

        def body(j, c):
            o = pl.multiple_of(j * r, r)
            acc[:, :n] += _dot(lhs[:, pl.ds(o, r)].astype(BF16), w[pl.ds(o, r), :])
            return c
        return body

    run(0, mm(xs, wq_v, rq, HQ * DH))
    for b in range(B):
        for h in range(HQ):
            qs[b * HQ + h:b * HQ + h + 1, :] = acc[b:b + 1, h * DH:(h + 1) * DH]

    run(1, mm(xs, w1_v, r1, F))
    h1 = acc[:, :F].astype(BF16).astype(F32)
    hs[...] = h1 * jax.nn.sigmoid(h1)

    def attn(n, c):
        o = pl.multiple_of(n * rep, rep)
        q = qs[pl.ds(o, rep), :].astype(BF16)
        s = lax.dot_general(q, k_v[n], (((1,), (1,)), ((), ())),
                            preferred_element_type=F32) * (DH ** -0.5)
        e = jnp.exp(s - jnp.max(s, axis=-1, keepdims=True))
        l = jnp.sum(e, axis=-1, keepdims=True)
        qs[pl.ds(o, rep), :] = _dot(e.astype(BF16), v_v[n]) / l
        return c
    run(2, attn, step=2)
    for b in range(B):
        for h in range(HQ):
            os_[b:b + 1, h * DH:(h + 1) * DH] = qs[b * HQ + h:b * HQ + h + 1, :]

    run(3, mm(hs, w2_v, r2, D))
    g = jax.nn.sigmoid(jnp.sum(xs[...] * gw_v[...].astype(F32).reshape(1, D), axis=-1, keepdims=True))
    hs[:, :D] = (1.0 - g) * acc[:, :D]
    run(4, mm(os_, wo_v, ro, D))
    out = g * acc[:, :D] + hs[:, :D]
    o_ref[...] = out[0:B].astype(o_ref.dtype)


def _call(A_x, A_k_cache, A_v_cache, A_wq, A_wo, B_w1, B_w2, gate_w,
          depth=3, rq=512, r1=512, ro=256, r2=896, compute=True):
    B, S, D = A_x.shape
    _, HKV, SK, _ = A_k_cache.shape
    F = B_w1.shape[1]
    W = min(4096, max(256, SK // 4))
    nsem = D // rq + D // r1 + 2 * B * HKV + F // r2 + HQ * DH // ro
    hbm = pl.BlockSpec(memory_space=pltpu.MemorySpace.HBM)
    V = pltpu.VMEM
    return pl.pallas_call(
        functools.partial(_kernel, depth=depth, rq=rq, r1=r1, ro=ro, r2=r2, compute=compute),
        in_specs=[hbm] * 8,
        out_specs=pl.BlockSpec(memory_space=pltpu.MemorySpace.VMEM),
        out_shape=jax.ShapeDtypeStruct((B * S, D), A_x.dtype),
        scratch_shapes=[
            V((B * S, D), BF16), V((D,), BF16),
            V((B * HKV, W, DH), BF16), V((B * HKV, W, DH), BF16),
            V(A_wq.shape, BF16), V(A_wo.shape, BF16), V(B_w1.shape, BF16), V(B_w2.shape, BF16),
            V((8, D), F32), V((8, HQ * DH), F32), V((B * HQ, DH), F32),
            V((8, HQ * DH), F32), V((8, F), F32),
            pltpu.SemaphoreType.DMA((nsem,)), pltpu.SemaphoreType.DMA((2,)),
        ],
        compiler_params=pltpu.CompilerParams(vmem_limit_bytes=100 * 1024 * 1024),
    )(A_x.reshape(B * S, D), A_k_cache, A_v_cache, A_wq, A_wo, B_w1, B_w2, gate_w).reshape(B, S, D)


@jax.jit
def pallas_gated_mix__sliding_block_cached__dense_activation_silu__decode_kernel(
    A_x, A_k_cache, A_v_cache, A_wq, A_wo, B_x, B_w1, B_w2, gate_w,
):
    del B_x
    return _call(A_x, A_k_cache, A_v_cache, A_wq, A_wo, B_w1, B_w2, gate_w)
```
